```python
import jax
import jax.numpy as jnp

def _softmax(x, axis=-1):
    return jax.nn.softmax(x, axis=axis)
def _gelu(x):
    return jax.nn.gelu(x, approximate=True)
def _silu(x):
    return jax.nn.silu(x)
def _sigmoid(x):
    return jax.nn.sigmoid(x)
def _layernorm(x, axis=-1, eps=1e-5):
    m = jnp.mean(x, axis=axis, keepdims=True)
    v = jnp.var(x, axis=axis, keepdims=True)
    return (x - m) / jnp.sqrt(v + eps)
def _scatter_add(tgt, idx, src, axis=0):
    return tgt.at[idx].add(src)
def _segment_sum(src, seg, n):
    return jax.ops.segment_sum(src, seg, n)
class _Rng:
    def __init__(self, key):
        self._k = key
    def _next(self):
        self._k, sub = jax.random.split(self._k)
        return sub
    def normal(self, shape):
        return jax.random.normal(self._next(), shape, dtype=jnp.bfloat16)
    def randint(self, lo, hi, shape):
        return jax.random.randint(self._next(), shape, lo, hi, dtype=jnp.int32)
    def uniform(self, shape, lo=0.0, hi=1.0):
        return jax.random.uniform(self._next(), shape, jnp.bfloat16, lo, hi)
    def permutation(self, n):
        return jax.random.permutation(self._next(), n)


kernel_name = 'sequential_preLN__compressed_kv_cla__moe_arch_mod__decode'

def setup_inputs():
    _rng = _Rng(jax.random.key(int.from_bytes(__import__("os").urandom(4), "little")))
    _w = (lambda a: (lambda t: t.astype(jnp.bfloat16) if jnp.issubdtype(t.dtype, jnp.floating) else t)(jnp.asarray(a)))
    def _A_setup():
        B, H, Sq, Sk, D, M = 1, 32, 1, 8192, 128, 512
        Dc = 4 * D
        return {
            "x": _w((lambda *s: _rng.normal(s) * 0.05)(B, Sq, M)),
            "c_kv": _w((lambda *s: _rng.normal(s) * 0.05)(B, Sk, Dc)),
            "w_q": _w((lambda *s: _rng.normal(s) * 0.05)(M, H, D) * (M ** -0.5)),
            "w_uk": _w((lambda *s: _rng.normal(s) * 0.05)(Dc, H, D) * (Dc ** -0.5)),
            "w_uv": _w((lambda *s: _rng.normal(s) * 0.05)(Dc, H, D) * (Dc ** -0.5)),
            "w_o": _w((lambda *s: _rng.normal(s) * 0.05)(H, D, M) * ((H * D) ** -0.5)),
        }
    _A_in = _A_setup()

    def _B_setup():
        B, S, D, F, C = 1, 1, 512, 1376, 1
        return {
            "x": _w((lambda *s: _rng.normal(s) * 0.05)(B, S, D)),
            "w_r": _w((lambda *s: _rng.normal(s) * 0.05)(D)),
            "w_gate": _w((lambda *s: _rng.normal(s) * 0.05)(D, F)),
            "w_up": _w((lambda *s: _rng.normal(s) * 0.05)(D, F)),
            "w_down": _w((lambda *s: _rng.normal(s) * 0.05)(F, D)),
        }
    _B_in = _B_setup()

    return {
        "A_x": _A_in["x"],
        "A_c_kv": _A_in["c_kv"],
        "A_w_q": _A_in["w_q"],
        "A_w_uk": _A_in["w_uk"],
        "A_w_uv": _A_in["w_uv"],
        "A_w_o": _A_in["w_o"],
        "B_x": _B_in["x"],
        "B_w_r": _B_in["w_r"],
        "B_w_gate": _B_in["w_gate"],
        "B_w_up": _B_in["w_up"],
        "B_w_down": _B_in["w_down"],
    }

def reference(A_x, A_c_kv, A_w_q, A_w_uk, A_w_uv, A_w_o, B_x, B_w_r, B_w_gate, B_w_up, B_w_down):
    def _A_ref(x, c_kv, w_q, w_uk, w_uv, w_o):
        B, Sq, M = x.shape[0], x.shape[1], x.shape[2]
        Sk = c_kv.shape[1]
        H, D = w_q.shape[1], w_q.shape[2]
        q = jnp.einsum("bqm,mhd->bhqd", x, w_q)
        k = jnp.einsum("bkc,chd->bhkd", c_kv, w_uk)
        v = jnp.einsum("bkc,chd->bhkd", c_kv, w_uv)
        scores = jnp.einsum("bhqd,bhkd->bhqk", q, k) * (D ** -0.5)
        off = Sk - Sq
        qi = jnp.arange(Sq)[:, None]
        kj = jnp.arange(Sk)[None, :]
        cmask = kj <= (qi + off)
        scores = jnp.where(cmask[None, None], scores, -1e9)
        p = _softmax(scores, axis=-1)
        ctx = jnp.einsum("bhqk,bhkd->bhqd", p, v)
        return jnp.einsum("bhqd,hdm->bqm", ctx, w_o)

    def _B_ref(x, w_r, w_gate, w_up, w_down):
        B, S, D = x.shape
        C = 1
        r = x @ w_r
        idx = jnp.argsort(-r, axis=-1)[:, :C]
        idx_e = jnp.repeat(idx.reshape(B, C, 1), D, axis=2)
        x_sel = jnp.take_along_axis(x, idx_e, axis=1)
        g = _silu(x_sel @ w_gate)
        u = x_sel @ w_up
        y = (g * u) @ w_down
        r_sel = _sigmoid(jnp.take_along_axis(r, idx, axis=1))
        y = y * r_sel.reshape(B, C, 1)
        b_off = (jnp.arange(B) * S).reshape(B, 1)
        flat_idx = (idx + b_off).reshape(B * C)
        zero = (x * 0.0).reshape(B * S, D)
        upd = _scatter_add(zero, flat_idx, y.reshape(B * C, D), axis=0)
        return x + upd.reshape(B, S, D)

    x = A_x
    h = x + _A_ref(_layernorm(x, axis=-1), A_c_kv, A_w_q, A_w_uk, A_w_uv, A_w_o)
    h2 = h + _B_ref(_layernorm(h, axis=-1), B_w_r, B_w_gate, B_w_up, B_w_down)
    return h2
```

```python
import functools
import jax
import jax.numpy as jnp
from jax import lax
from jax.experimental import pallas as pl
from jax.experimental.pallas import tpu as pltpu

H, D, M, DC, SK, F = 32, 128, 512, 512, 8192, 1376
FP = 1408
BF, F32 = jnp.bfloat16, jnp.float32
NT = (((1,), (1,)), ((), ()))


def _ln(v):
    m = jnp.mean(v, axis=-1, keepdims=True)
    c = v - m
    var = jnp.mean(c * c, axis=-1, keepdims=True)
    return c / jnp.sqrt(var + 1e-5)


def build(ck=1024, n_ckv=4, n_wo=2, dsplit=(768, 512, 96), T=8, dma=True, stages="123456"):
    def kern(x_hbm, ckv_hbm, wq_hbm, wuk_hbm, wuv_hbm, wo_hbm, wr_hbm, wg_hbm, wu_hbm, wd_hbm, out_hbm,
             x_v, wr_v, ckv_v, wq_v, wuk_v, wuv_v, wo_v, wg_v, wu_v, wd_v, out_v, r_v, ctx_v, sems):
        cps = []

        def add(src, dst):
            c = pltpu.make_async_copy(src, dst, sems.at[len(cps)])
            cps.append(c)
            return c

        c_x = add(x_hbm, x_v)
        c_q = add(wq_hbm, wq_v)
        c_r = add(wr_hbm, wr_v)
        c_uk = add(wuk_hbm, wuk_v)
        rows = SK // n_ckv
        c_kv = [add(ckv_hbm.at[0, pl.ds(i * rows, rows)], ckv_v.at[pl.ds(i * rows, rows)]) for i in range(n_ckv)]
        c_uv = add(wuv_hbm, wuv_v)
        hh = H // n_wo
        c_o = [add(wo_hbm.at[pl.ds(i * hh, hh)], wo_v.at[pl.ds(i * hh, hh)]) for i in range(n_wo)]
        c_g = add(wg_hbm, wg_v.at[pl.ds(0, F)])
        c_u = add(wu_hbm, wu_v.at[pl.ds(0, F)])
        c_d, o = [], 0
        for n in dsplit:
            c_d.append(add(wd_hbm.at[pl.ds(o, n)], wd_v.at[pl.ds(o, n)]))
            o += n
        assert o == F
        if dma:
            for c in cps:
                c.start()
        wait = (lambda c: c.wait()) if dma else (lambda c: None)

        zpad = jnp.zeros((FP - F, M), BF)
        wg_v[pl.ds(F, FP - F), :] = zpad
        wu_v[pl.ds(F, FP - F), :] = zpad
        wd_v[pl.ds(F, FP - F), :] = zpad

        row = lax.broadcasted_iota(jnp.int32, (H, 128), 0)
        lane = lax.broadcasted_iota(jnp.int32, (H, 128), 1)
        diag = (lane % H) == row
        sub8 = lax.broadcasted_iota(jnp.int32, (8, 128), 0)

        def head_contract(a, w_v):
            stack = jnp.concatenate([a[:, j * 128:(j + 1) * 128] for j in range(4)], axis=0)
            r_v[...] = stack.T

            def body(i, acc):
                t0 = pl.multiple_of(i * T, T)
                rr = r_v[pl.ds(t0, T), :]
                for s in range(T):
                    lhs = jnp.where(diag, rr[s:s + 1, :], 0.0).astype(BF)
                    tile = w_v[:, t0 + s].reshape(128, 128)
                    acc = acc + jnp.dot(lhs, tile, preferred_element_type=F32)
                return acc

            return lax.fori_loop(0, 128 // T, body, jnp.zeros((H, D), F32))

        wait(c_x)
        x = x_v[0].astype(F32)
        xn = _ln(x)
        wait(c_q)
        if "1" in stages:
            q = head_contract(jnp.broadcast_to(xn, (H, M)), wq_v)
        else:
            q = jnp.broadcast_to(xn[:, :128], (H, D))
        qb = q.astype(BF)

        wait(c_r)
        wait(c_uk)

        def body2(i, carry):
            t0 = pl.multiple_of(i * T, T)
            for g in range(T // 8):
                merged = jnp.zeros((8, 128), F32)
                for s in range(8):
                    tile = wuk_v[:, t0 + g * 8 + s].reshape(128, 128)
                    o = lax.dot_general(qb, tile, NT, preferred_element_type=F32)
                    rs = jnp.sum(jnp.where(diag, o, 0.0), axis=0, keepdims=True)
                    merged = jnp.where(sub8 == s, rs, merged)
                r_v[pl.ds(t0 + g * 8, 8), :] = merged
            return carry

        if "2" in stages:
            lax.fori_loop(0, 128 // T, body2, 0)
        rt = r_v[...].T * (D ** -0.5)
        ql = jnp.concatenate([rt[j * H:(j + 1) * H, :] for j in range(4)], axis=1).astype(BF)

        def body3(i, carry):
            m, l, acc = carry
            c = ckv_v[pl.ds(pl.multiple_of(i * ck, ck), ck), :]
            s = lax.dot_general(ql, c, NT, preferred_element_type=F32)
            m_new = jnp.maximum(m, jnp.max(s, axis=-1, keepdims=True))
            alpha = jnp.exp(m - m_new)
            p = jnp.exp(s - m_new)
            l = alpha * l + jnp.sum(p, axis=-1, keepdims=True)
            acc = alpha * acc + jnp.dot(p.astype(BF), c, preferred_element_type=F32)
            return m_new, l, acc

        carry = (jnp.full((H, 1), -jnp.inf, F32), jnp.zeros((H, 1), F32), jnp.zeros((H, DC), F32))
        per = rows // ck
        for b in range(n_ckv):
            wait(c_kv[b])
            if "3" in stages:
                carry = lax.fori_loop(b * per, (b + 1) * per, body3, carry)
        _, l, acc = carry
        cl = acc / l

        wait(c_uv)
        if "4" in stages:
            ctx = head_contract(cl, wuv_v)
        else:
            ctx = cl[:, :128]
        ctx_v[...] = ctx

        def body5(i, acc):
            h0 = pl.multiple_of(i * 8, 8)
            cc = ctx_v[pl.ds(h0, 8), :]
            for s in range(8):
                lhs = jnp.broadcast_to(cc[s:s + 1, :], (16, D)).astype(BF)
                acc = acc + jnp.dot(lhs, wo_v[h0 + s], preferred_element_type=F32)
            return acc

        a = jnp.zeros((16, M), F32)
        for b in range(n_wo):
            wait(c_o[b])
            if "5" in stages:
                a = lax.fori_loop(b * hh // 8, (b + 1) * hh // 8, body5, a)
        hres = x + a[0:1, :]
        hn = _ln(hres)
        wr = wr_v[...].astype(F32)
        wr = jnp.concatenate([wr[j:j + 1, :] for j in range(4)], axis=1)
        r = jnp.sum(hn * wr, axis=-1, keepdims=True)
        gate = jax.nn.sigmoid(r)
        hb = jnp.broadcast_to(hn, (16, M)).astype(BF)
        wait(c_g)
        g = lax.dot_general(hb, wg_v[...], NT, preferred_element_type=F32)
        g = g * jax.nn.sigmoid(g)
        wait(c_u)
        u = lax.dot_general(hb, wu_v[...], NT, preferred_element_type=F32)
        act = (g * u).astype(BF)
        y = jnp.zeros((16, M), F32)
        o = 0
        for c, n in zip(c_d, dsplit):
            wait(c)
            n = (n + 127) // 128 * 128
            y = y + jnp.dot(act[:, o:o + n], wd_v[pl.ds(o, n), :], preferred_element_type=F32)
            o += n
        res = hres + (hn + (hn * 0.0 + y[0:1, :] * gate))
        out_v[0] = res.astype(BF)
        co = pltpu.make_async_copy(out_v, out_hbm, sems.at[len(cps)])
        co.start()
        co.wait()

    @jax.jit
    def f(A_x, A_c_kv, A_w_q, A_w_uk, A_w_uv, A_w_o, B_x, B_w_r, B_w_gate, B_w_up, B_w_down):
        w4 = lambda w: w.reshape(4, 128, H, D)
        return pl.pallas_call(
            kern,
            out_shape=jax.ShapeDtypeStruct((1, 1, M), BF),
            in_specs=[pl.BlockSpec(memory_space=pl.ANY)] * 10,
            out_specs=pl.BlockSpec(memory_space=pl.ANY),
            scratch_shapes=[
                pltpu.VMEM((1, 1, M), BF), pltpu.VMEM((4, 128), BF), pltpu.VMEM((SK, DC), BF),
                pltpu.VMEM((4, 128, H, D), BF), pltpu.VMEM((4, 128, H, D), BF), pltpu.VMEM((4, 128, H, D), BF),
                pltpu.VMEM((H, D, M), BF),
                pltpu.VMEM((FP, M), BF), pltpu.VMEM((FP, M), BF), pltpu.VMEM((FP, M), BF),
                pltpu.VMEM((1, 1, M), BF), pltpu.VMEM((128, 128), F32), pltpu.VMEM((H, D), F32),
                pltpu.SemaphoreType.DMA((32,)),
            ],
            compiler_params=pltpu.CompilerParams(vmem_limit_bytes=100 * 2**20),
        )(A_x, A_c_kv, w4(A_w_q), w4(A_w_uk), w4(A_w_uv), A_w_o, B_w_r.reshape(4, 128), B_w_gate.T, B_w_up.T, B_w_down)

    return f


pallas_sequential_preLN__compressed_kv_cla__moe_arch_mod__decode_kernel = build()
```

```python
import jax
import jax.numpy as jnp
from jax import lax
from jax.experimental import pallas as pl
from jax.experimental.pallas import tpu as pltpu

H, D, M, DC, SK, F = 32, 128, 512, 512, 8192, 1376
BF, F32 = jnp.bfloat16, jnp.float32
NT = (((1,), (1,)), ((), ()))
NF = pl.cdiv(F, 128)


def _layernorm(v):
    c = v - jnp.mean(v, axis=-1, keepdims=True)
    var = jnp.mean(c * c, axis=-1, keepdims=True)
    return c / jnp.sqrt(var + 1e-5)


def _aligned(i, n):
    return i if isinstance(i, int) else pl.multiple_of(i, n)


def build(W1=8, W0=8, forder=(0, 6, 1, 7, 2, 8, 3, 9, 4, 5, 10), compute=True, nochk=True, only=None, G=4):
    def body(x_hbm, ckv_hbm, wq_hbm, wuk_hbm, wuv_hbm, wo_hbm, wr_hbm, wg_hbm, wu_hbm, wd_hbm, out_ref,
             x_v, wr_v, ckv_v, wq_v, wuk_v, wuv_v, wo_v, wg_v, wu_v, wd_v, r_v, ctx_v, sems):
        def head_unit(src, dst):
            def unit(c, d):
                t0, u = (c % 2) * 64 + (c // 2) * 4 + d * 4, c + 2 * d
                return ((src.at[pl.ds(0, 3), pl.ds(t0, 4)], dst.at[u, pl.ds(0, 3)]),
                        (src.at[pl.ds(3, 1), pl.ds(t0, 4)], dst.at[u, pl.ds(3, 1)]))
            return unit

        def row_start(c, d):
            return _aligned((c % 2) * 512 + (c // 2) * 32 + d * 32, 32)

        def ckv_unit(a):
            def unit(c, d):
                r0, u = row_start(c, d), a * 32 + c + 2 * d
                return ((ckv_hbm.at[a, pl.ds(0, 3), pl.ds(r0, 32)], ckv_v.at[u, pl.ds(0, 3)]),
                        (ckv_hbm.at[a, pl.ds(3, 1), pl.ds(r0, 32)], ckv_v.at[u, pl.ds(3, 1)]))
            return unit

        def wo_unit(c, d):
            r0 = row_start(c, d)
            return ((wo_hbm.at[pl.ds(0, 3), pl.ds(r0, 32)], wo_v.at[pl.ds(0, 3), pl.ds(r0, 32)]),
                    (wo_hbm.at[pl.ds(3, 1), pl.ds(r0, 32)], wo_v.at[pl.ds(3, 1), pl.ds(r0, 32)]))

        def ffn_rows(n):
            return n * 128, min(128, F - n * 128)

        def ffn_unit(u, _):
            if u < 2 * NF:
                src, dst = ((wg_hbm, wg_v), (wu_hbm, wu_v))[u % 2]
                r0, n = ffn_rows(forder[u // 2])
            else:
                src, dst = wd_hbm, wd_v
                r0, n = ffn_rows(forder[u - 2 * NF])
            lo, hi = pl.ds(r0, n - 32), pl.ds(r0 + n - 32, 32)
            return (src.at[lo], dst.at[lo]), (src.at[hi], dst.at[hi])

        segments = ((32, head_unit(wq_hbm, wq_v)), (32, head_unit(wuk_hbm, wuk_v)),
                    (32, ckv_unit(0)), (32, ckv_unit(1)),
                    (32, head_unit(wuv_hbm, wuv_v)), (32, wo_unit), (3 * NF, ffn_unit))
        n_units = sum(n for n, _ in segments)

        def locate(g):
            base = 0
            for k, (n, _) in enumerate(segments):
                if g < base + n:
                    return k, base
                base += n
            return None, base

        def copy(g, d, part):
            k, base = locate(g)
            src, dst = segments[k][1](g - base, d)[part]
            return pltpu.make_async_copy(src, dst, sems.at[g + 2 * d])

        def arrive(g, d=0):
            copy(g, d, 0).wait()
            copy(g, d, 1).wait()

        def refill(g, d=0):
            if g + W1 < n_units:
                copy(g + W1, d, 0).start(priority=1)
            if g + W0 < n_units:
                copy(g + W0, d, 1).start(priority=0)

        def step(g, d=0):
            arrive(g, d)
            refill(g, d)

        def stage(g0, n_iter, per, fn, carry):
            def key(i):
                segs = tuple(locate(g0 + i * per + k + w)[0] for k in range(per) for w in (0, W0, W1))
                return i if len(segments) - 1 in segs else segs
            i = 0
            while i < n_iter:
                j = i + 1
                while j < n_iter and key(j) == key(i):
                    j += 1
                if j - i == 1:
                    carry = fn(i, lambda k, i=i: (g0 + i * per + k, 0), carry)
                else:
                    carry = lax.fori_loop(
                        i, j, lambda t, c, i=i: fn(t, lambda k: (g0 + i * per + k, (t - i) * (per // 2)), c), carry)
                i = j
            return carry

        small = (pltpu.make_async_copy(x_hbm, x_v, sems.at[n_units]),
                 pltpu.make_async_copy(wr_hbm, wr_v, sems.at[n_units + 1]))
        copy(0, 0, 0).start(priority=1)
        for c in small:
            c.start()
        for g in range(max(W0, W1)):
            if 0 < g < W1:
                copy(g, 0, 0).start(priority=1)
            if g < W0:
                copy(g, 0, 1).start(priority=0)

        row = lax.broadcasted_iota(jnp.int32, (H, 128), 0)
        lane = lax.broadcasted_iota(jnp.int32, (H, 128), 1)
        diag = (lane % H) == row
        sub8 = lax.broadcasted_iota(jnp.int32, (8, 128), 0)

        def tile(w_v, u, s):
            return w_v[u, :, s].reshape(4 * H, D)

        def spread(a):
            r_v[...] = jnp.concatenate([a[:, j * 128:(j + 1) * 128] for j in range(4)], axis=0).T

        def head_contract(w_v, compute=compute):
            def fn(i, at, acc):
                rows = [r_v[pl.ds(_aligned(p * 64 + i * 8, 8), 8), :] for p in range(2)]
                for k in range(4):
                    step(*at(k))
                    for s in range(4 if compute else 0):
                        t = (k // 2) * 4 + s
                        lhs = jnp.where(diag, rows[k % 2][t:t + 1, :], 0.0).astype(BF)
                        acc = acc + jnp.dot(lhs, tile(w_v, i * 4 + k, s), preferred_element_type=F32)
                return acc
            return fn

        for c in small:
            c.wait()
        x = x_v[0].astype(F32)
        spread(jnp.broadcast_to(_layernorm(x), (H, M)))
        q = stage(0, 8, 4, head_contract(wq_v, compute and only in (None, 1)), jnp.zeros((H, D), F32)).astype(BF)

        def absorb(i, at, carry):
            merged = [jnp.zeros((8, 128), F32)] * 2
            for k in range(4):
                step(*at(k))
                for s in range(4 if compute and only in (None, 2) else 0):
                    o = lax.dot_general(q, tile(wuk_v, i * 4 + k, s), NT, preferred_element_type=F32)
                    picked = jnp.sum(jnp.where(diag, o, 0.0), axis=0, keepdims=True)
                    merged[k % 2] = jnp.where(sub8 == (k // 2) * 4 + s, picked, merged[k % 2])
            for p in range(2):
                r_v[pl.ds(_aligned(p * 64 + i * 8, 8), 8), :] = merged[p]
            return carry

        stage(32, 8, 4, absorb, 0)
        rt = r_v[...].T * (D ** -0.5)
        ql = jnp.concatenate([rt[j * H:(j + 1) * H, :] for j in range(4)], axis=1).astype(BF)

        def keys(u):
            return ckv_v[u].reshape(128, DC)

        def scores(u):
            return lax.dot_general(ql, keys(u), NT, preferred_element_type=F32)

        def softmax_update(s, m, l):
            top = s[0]
            for v in s[1:]:
                top = jnp.maximum(top, v)
            m_new = jnp.maximum(m, jnp.max(top, axis=-1, keepdims=True))
            alpha = jnp.exp(m - m_new)
            p = [jnp.exp(v - m_new) for v in s]
            l = alpha * l
            for v in p:
                l = l + v
            return [v.astype(BF) for v in p], alpha, m_new, l

        def attend(i, at, carry):
            s, m, l, acc = carry
            for k in range(G):
                arrive(*at(k))
            s_next = []
            for k in range(G):
                if k % 2 == 0:
                    refill(*at(k // 2))
                s_next.append(scores((i + 1) * G + k))
            p, alpha, m, l = softmax_update(s, m, l)
            acc = alpha * acc
            for k in range(G):
                if k % 2 == 0:
                    refill(*at(G // 2 + k // 2))
                acc = acc + jnp.dot(p[k], keys(i * G + k), preferred_element_type=F32)
            return tuple(s_next), m, l, acc

        s = []
        for k in range(G):
            step(64 + k)
            s.append(scores(k))
        carry = (tuple(s), jnp.full((H, 1), -jnp.inf, F32), jnp.zeros((H, 128), F32), jnp.zeros((H, DC), F32))
        s, m, l, acc = stage(64 + G, 64 // G - 1, G, attend, carry)
        step(128)
        p, alpha, m, l = softmax_update(s, m, l)
        acc = alpha * acc
        for k in range(G):
            if k in (0, G // 2):
                step(129 + (k > 0))
            acc = acc + jnp.dot(p[k], keys(64 - G + k), preferred_element_type=F32)
        step(131)
        spread(acc / jnp.sum(l, axis=-1, keepdims=True))
        ctx_v[...] = stage(132, 8, 4, head_contract(wuv_v, compute and only in (None, 4)), jnp.zeros((H, D), F32))

        def project(g, at, acc):
            for k in range(8):
                step(*at(k))
                if compute and only in (None, 5):
                    lhs = jnp.broadcast_to(ctx_v[pl.ds(4 * k + g, 1), :], (16, D)).astype(BF)
                    w = wo_v[k // 2, pl.ds(_aligned((k % 2) * 512 + g * 128, 128), 128), :]
                    acc = acc + jnp.dot(lhs, w, preferred_element_type=F32)
            return acc

        for g in range(164, 168):
            step(g)
        attn = stage(168, 3, 8, project, jnp.zeros((16, M), F32))
        attn = project(3, lambda k: (192 + k, 0), attn)

        h = x + attn[0:1, :]
        hn = _layernorm(h)
        wr = wr_v[...].astype(F32)
        wr = jnp.concatenate([wr[j:j + 1, :] for j in range(4)], axis=1)
        gate = jax.nn.sigmoid(jnp.sum(hn * wr, axis=-1, keepdims=True))
        hb = jnp.broadcast_to(hn, (16, M)).astype(BF)

        act, g = [], 200
        for j in range(NF):
            while g <= max(200 + j, 192 + 2 * j + 1):
                step(g)
                g += 1
            rows = pl.ds(*ffn_rows(forder[j]))
            gj = lax.dot_general(hb, wg_v[rows, :], NT, preferred_element_type=F32)
            uj = lax.dot_general(hb, wu_v[rows, :], NT, preferred_element_type=F32)
            act.append((gj * jax.nn.sigmoid(gj) * uj).astype(BF))
        y = jnp.zeros((16, M), F32)
        for j in range(NF):
            step(192 + 2 * NF + j)
            y = y + jnp.dot(act[j], wd_v[pl.ds(*ffn_rows(forder[j])), :], preferred_element_type=F32)
        out_ref[0] = (h + (hn + (hn * 0.0 + y[0:1, :] * gate))).astype(out_ref.dtype)

    def kern(*refs):
        pl.run_scoped(lambda sems: body(*refs, sems), pltpu.SemaphoreType.DMA((192 + 3 * NF + 2,)))

    @jax.jit
    def run(A_x, A_c_kv, A_w_q, A_w_uk, A_w_uv, A_w_o, B_x, B_w_r, B_w_gate, B_w_up, B_w_down):
        del B_x
        quarters = lambda w: w.reshape(4, DC // 4, H, D)
        head_buf = pltpu.VMEM((32, 4, 4, H, D), BF)
        return pl.pallas_call(
            kern,
            out_shape=jax.ShapeDtypeStruct((1, 1, M), A_x.dtype),
            in_specs=[pl.BlockSpec(memory_space=pl.ANY)] * 10,
            out_specs=pl.BlockSpec(memory_space=pltpu.VMEM),
            scratch_shapes=[
                pltpu.VMEM((1, 1, M), BF), pltpu.VMEM((4, 128), BF), pltpu.VMEM((64, 4, 32, DC), BF),
                head_buf, head_buf, head_buf, pltpu.VMEM((4, 1024, M), BF),
                pltpu.VMEM((F, M), BF), pltpu.VMEM((F, M), BF), pltpu.VMEM((F, M), BF),
                pltpu.VMEM((128, 128), F32), pltpu.VMEM((H, D), F32),
            ],
            compiler_params=pltpu.CompilerParams(vmem_limit_bytes=64 * 2**20, disable_bounds_checks=nochk),
        )(A_x, A_c_kv.reshape(2, 4, SK // 8, DC), quarters(A_w_q), quarters(A_w_uk), quarters(A_w_uv),
          A_w_o.reshape(4, H * D // 4, M), B_w_r.reshape(4, 128), B_w_gate.T, B_w_up.T, B_w_down)

    return run


pallas_sequential_preLN__compressed_kv_cla__moe_arch_mod__decode_kernel = build(W1=16, W0=8, nochk=False)
```

```python
import jax
import jax.numpy as jnp
from jax import lax
from jax.experimental import pallas as pl
from jax.experimental.pallas import tpu as pltpu

H, D, M, DC, SK, F = 32, 128, 512, 512, 8192, 1376
BF, F32 = jnp.bfloat16, jnp.float32
NT = (((1,), (1,)), ((), ()))
NF = pl.cdiv(F, 128)
FT = F // 4 - 32 * (NF - 1)


def _layernorm(v):
    c = v - jnp.mean(v, axis=-1, keepdims=True)
    var = jnp.mean(c * c, axis=-1, keepdims=True)
    return c / jnp.sqrt(var + 1e-5)


def _aligned(i, n):
    return i if isinstance(i, int) else pl.multiple_of(i, n)


def build(W1=16, W0=6, forder=(0, 5, 1, 6, 2, 7, 3, 8, 4, 9, 10), compute=True, nochk=False, only=None, G=4, puredma=False, nun=None, bulk=0, RM=8, vtail=True):
    def body(x_hbm, ckv_hbm, wq_hbm, wuk_hbm, wuv_hbm, wo_hbm, wr_hbm, wg_hbm, wu_hbm, wd_hbm, out_ref,
             x_v, wr_v, ckv_v, wq_v, wuk_v, wuv_v, wo_v, wg_v, wu_v, wd_v, tail_v, r_v, ctx_v, sems):
        def head_unit(src, dst):
            def unit(c, d):
                t0, u = (c % 2) * 64 + (c // 2) * 4 + d * 4, c + 2 * d
                return ((src.at[pl.ds(0, 3), pl.ds(t0, 4)], dst.at[u, pl.ds(0, 3)]),
                        (src.at[pl.ds(3, 1), pl.ds(t0, 4)], dst.at[u, pl.ds(3, 1)]))
            return unit

        def ckv_unit(c, d):
            e, u = c // 2 + d, c + 2 * d
            r0 = _aligned((c % 2) * 512 + (e & 1) * 1024 + (e >> 1) * 32, 32)
            return ((ckv_hbm.at[pl.ds(0, 3), pl.ds(r0, 32)], ckv_v.at[u, pl.ds(0, 3)]),
                    (ckv_hbm.at[pl.ds(3, 1), pl.ds(r0, 32)], ckv_v.at[u, pl.ds(3, 1)]))

        def wo_unit(c, d):
            r0, u = _aligned((c % 2) * 512 + (c // 2) * 32 + d * 32, 32), c + 2 * d
            return ((wo_hbm.at[pl.ds(0, 3), pl.ds(r0, 32)], wo_v.at[u, pl.ds(0, 3)]),
                    (wo_hbm.at[pl.ds(3, 1), pl.ds(r0, 32)], wo_v.at[u, pl.ds(3, 1)]))

        def ffn_unit(u, _):
            src, dst, tail = ffn[u % 2] if u < 2 * NF else ffn[2]
            j = forder[u // 2 if u < 2 * NF else u - 2 * NF]
            if j < NF - 1:
                rows = pl.ds(j * 32, 32)
                return ((src.at[pl.ds(0, 3), rows], dst.at[j, pl.ds(0, 3)]),
                        (src.at[pl.ds(3, 1), rows], dst.at[j, pl.ds(3, 1)]))
            return tuple((src.at[k, pl.ds(j * 32, FT)], tail.at[pl.ds(k * FT, FT)]) for k in range(4))

        def ffn_tile(w, j):
            _, dst, tail = ffn[w]
            return dst[forder[j]].reshape(128, M) if forder[j] < NF - 1 else tail[...]

        ffn = ((wg_hbm, wg_v, tail_v.at[0]), (wu_hbm, wu_v, tail_v.at[1]), (wd_hbm, wd_v, tail_v.at[2]))
        segments = ((32, head_unit(wq_hbm, wq_v)), (32, head_unit(wuk_hbm, wuk_v)),
                    (64, ckv_unit),
                    (32, head_unit(wuv_hbm, wuv_v)), (32, wo_unit), (3 * NF, ffn_unit))
        n_units = nun or sum(n for n, _ in segments)

        def locate(g):
            base = 0
            for k, (n, _) in enumerate(segments):
                if g < base + n:
                    return k, base
                base += n
            return None, base

        def copies(g, d=0):
            k, base = locate(g)
            split = g == n_units - 1
            return [pltpu.make_async_copy(src, dst, sems.at[g + 2 * d + (n if split else 0)])
                    for n, (src, dst) in enumerate(segments[k][1](g - base, d))]

        def start_low(g, d=0):
            for c in copies(g, d)[:-1]:
                c.start(priority=1)

        def start_high(g, d=0):
            copies(g, d)[-1].start(priority=0)

        def arrive(g, d=0):
            for c in copies(g, d):
                c.wait()

        def refill(g, d=0):
            if g + W0 < n_units:
                start_high(g + W0, d)
            if g + W1 < n_units:
                start_low(g + W1, d)

        def step(g, d=0):
            arrive(g, d)
            refill(g, d)

        def stage(g0, n_iter, per, fn, carry):
            def key(i):
                segs = tuple(locate(g0 + i * per + k + w)[0] for k in range(per) for w in (0, W0, W1))
                return i if len(segments) - 1 in segs else segs
            i = 0
            while i < n_iter:
                j = i + 1
                while j < n_iter and key(j) == key(i):
                    j += 1
                if j - i == 1:
                    carry = fn(i, lambda k, i=i: (g0 + i * per + k, 0), carry)
                else:
                    carry = lax.fori_loop(
                        i, j, lambda t, c, i=i: fn(t, lambda k: (g0 + i * per + k, (t - i) * (per // 2)), c), carry)
                i = j
            return carry

        small = (pltpu.make_async_copy(x_hbm, x_v, sems.at[n_units + 3]),
                 pltpu.make_async_copy(wr_hbm, wr_v, sems.at[n_units + 4]))
        start_low(0)
        for c in small:
            c.start()
        for g in range(max(W0, W1)):
            if 0 < g < W1:
                start_low(g)
            if g < W0:
                copies(g)[-1].start(priority=1)

        if puredma:
            for c in small:
                c.wait()
            def fn(i, at, c):
                for k in range(4):
                    step(*at(k))
                return c
            if bulk:
                ctx_v[...] = jnp.zeros((H, D), F32)
                for g in range(192):
                    step(g)
                    v = ctx_v[0:8, :]
                    for _ in range(bulk - 1):
                        v = v * 1.0001 + 0.5
                    ctx_v[0:8, :] = v
            else:
                stage(0, min(n_units, 192) // 4, 4, fn, 0)
            for g in range(192, n_units):
                step(g)
            out_ref[0] = x_v[0] + (ctx_v[0:1, 0:1].astype(BF) if bulk else 0)
            return
        row = lax.broadcasted_iota(jnp.int32, (H, 128), 0)
        lane = lax.broadcasted_iota(jnp.int32, (H, 128), 1)
        diag = (lane % H) == row
        sub8 = lax.broadcasted_iota(jnp.int32, (8, 128), 0)

        def tile(w_v, u, s):
            return w_v[u, :, s].reshape(4 * H, D)

        def spread(a):
            r_v[...] = jnp.concatenate([a[:, j * 128:(j + 1) * 128] for j in range(4)], axis=0).T

        def head_contract(w_v, compute=compute):
            def fn(i, at, acc):
                rows = [r_v[pl.ds(_aligned(p * 64 + i * 8, 8), 8), :] for p in range(2)]
                for k in range(4):
                    step(*at(k))
                    for s in range(4 if compute else 0):
                        t = (k // 2) * 4 + s
                        lhs = jnp.where(diag, rows[k % 2][t:t + 1, :], 0.0).astype(BF)
                        acc = acc + jnp.dot(lhs, tile(w_v, i * 4 + k, s), preferred_element_type=F32)
                return acc
            return fn

        for c in small:
            c.wait()
        x = x_v[0].astype(F32)
        spread(jnp.broadcast_to(_layernorm(x), (H, M)))
        q = stage(0, 8, 4, head_contract(wq_v, compute and only in (None, 1)), jnp.zeros((H, D), F32)).astype(BF)

        def absorb(i, at, carry):
            merged = [jnp.zeros((8, 128), F32)] * 2
            for k in range(4):
                step(*at(k))
                for s in range(4 if compute and only in (None, 2) else 0):
                    o = lax.dot_general(q, tile(wuk_v, i * 4 + k, s), NT, preferred_element_type=F32)
                    picked = jnp.sum(jnp.where(diag, o, 0.0), axis=0, keepdims=True)
                    merged[k % 2] = jnp.where(sub8 == (k // 2) * 4 + s, picked, merged[k % 2])
            for p in range(2):
                r_v[pl.ds(_aligned(p * 64 + i * 8, 8), 8), :] = merged[p]
            return carry

        stage(32, 8, 4, absorb, 0)
        step(64)
        rt = r_v[...].T * (D ** -0.5)
        ql = jnp.concatenate([rt[j * H:(j + 1) * H, :] for j in range(4)], axis=1).astype(BF)

        def keys(u):
            return ckv_v[u].reshape(128, DC)

        def scores(u):
            return lax.dot_general(ql, keys(u), NT, preferred_element_type=F32)

        def softmax_update(s, m, l):
            top = s[0]
            for v in s[1:]:
                top = jnp.maximum(top, v)
            m_new = jnp.maximum(m, jnp.max(top, axis=-1, keepdims=True))
            alpha = jnp.exp(m - m_new)
            p = [jnp.exp(v - m_new) for v in s]
            l = alpha * l
            for v in p:
                l = l + v
            return [v.astype(BF) for v in p], alpha, m_new, l

        def attend(i, at, carry):
            s, m, l, acc = carry
            step(*at(0))
            if only not in (None, 3):
                step(*at(1))
                return carry
            s_next = (scores(2 * i + 2), scores(2 * i + 3))
            p, alpha, m, l = softmax_update(s, m, l)
            acc = alpha * acc
            step(*at(1))
            for k in range(2):
                acc = acc + jnp.dot(p[k], keys(2 * i + k), preferred_element_type=F32)
            return s_next, m, l, acc

        step(65)
        s0 = scores(0)
        step(66)
        carry = ((s0, scores(1)), jnp.full((H, 1), -jnp.inf, F32), jnp.zeros((H, 128), F32), jnp.zeros((H, DC), F32))
        s, m, l, acc = stage(67, 31, 2, attend, carry)
        step(129)
        p, alpha, m, l = softmax_update(s, m, l)
        acc = alpha * acc
        step(130)
        for k in range(2):
            acc = acc + jnp.dot(p[k], keys(62 + k), preferred_element_type=F32)
        step(131)
        spread(acc / jnp.sum(l, axis=-1, keepdims=True))
        ctx = stage(132, 8, 4, head_contract(wuv_v), jnp.zeros((H, D), F32))

        step(164)
        for i in range(4):
            ctx_v[8 * i:8 * i + 8, :] = jnp.concatenate(
                [ctx[8 * j:8 * j + 8, 32 * i:32 * i + 32] for j in range(4)], axis=1)

        def project(g, at, acc):
            for k in range(8):
                step(*at(k))
                if compute and only in (None, 5):
                    lhs = jnp.broadcast_to(ctx_v[pl.ds(4 * k + g, 1), :], (RM, 128)).astype(BF)
                    acc = acc + jnp.dot(lhs, wo_v[8 * g + k].reshape(128, M), preferred_element_type=F32)
            return acc

        attn = stage(165, 4, 8, project, jnp.zeros((RM, M), F32))
        step(197)
        h = x + attn[0:1, :]
        hc = h - jnp.mean(h, axis=-1, keepdims=True)
        step(198)
        hn = hc / jnp.sqrt(jnp.mean(hc * hc, axis=-1, keepdims=True) + 1e-5)
        hb = jnp.broadcast_to(hn, (RM, M)).astype(BF)
        step(199)
        wr = wr_v[...].astype(F32)
        wr = jnp.concatenate([wr[j:j + 1, :] for j in range(4)], axis=1)
        gate = jax.nn.sigmoid(jnp.sum(hn * wr, axis=-1, keepdims=True))

        act, pre, g = [], None, 200
        for j in range(NF + 1):
            while g <= max(200 + j, 192 + min(2 * j + 1, 2 * NF)):
                step(g)
                g += 1
            if pre is not None:
                act.append(pre[0] * jax.nn.sigmoid(pre[0]) * pre[1])
            if j < NF:
                pre = [lax.dot_general(hb, ffn_tile(w, j), NT, preferred_element_type=F32) for w in range(2)]
        y = jnp.zeros((RM, M), F32)
        last = act[-1][0:1, :]
        if vtail:
            col = jnp.concatenate([last, jnp.zeros((1, 128 - 4 * FT), F32)], axis=1)
            col = jnp.broadcast_to(col, (128, 128)).T
        for j in range(NF - 1):
            if j > 0:
                step(192 + 2 * NF + j)
            y = y + jnp.dot(act[j].astype(BF), ffn_tile(2, j), preferred_element_type=F32)
        res = h + (hn + (hn * 0.0 + y[0:1, :] * gate))
        if vtail:
            part = jnp.zeros((8, M), F32)
            pieces = copies(n_units - 1)
            for k in (3, 0, 1, 2):
                pieces[k].wait()
                for r in range(k * FT, (k + 1) * FT, 8):
                    a = jnp.concatenate([col[r:r + 8, :]] * (M // 128), axis=1)
                    part = part + a * tail_v[2, r:r + 8, :].astype(F32)
            y = jnp.sum(part, axis=0, keepdims=True)
        else:
            step(n_units - 1)
            y = jnp.dot(act[-1].astype(BF), ffn_tile(2, NF - 1), preferred_element_type=F32)[0:1, :]
        out_ref[0] = (res + y * gate).astype(out_ref.dtype)

    def kern(*refs):
        pl.run_scoped(lambda sems: body(*refs, sems), pltpu.SemaphoreType.DMA((192 + 3 * NF + 5,)))

    @jax.jit
    def run(A_x, A_c_kv, A_w_q, A_w_uk, A_w_uv, A_w_o, B_x, B_w_r, B_w_gate, B_w_up, B_w_down):
        del B_x
        quarters = lambda w: w.reshape(4, DC // 4, H, D)
        head_buf = pltpu.VMEM((32, 4, 4, H, D), BF)
        ffn_buf = pltpu.VMEM((NF - 1, 4, 32, M), BF)
        ffn_view = lambda w: w.reshape(4, F // 4, M)
        return pl.pallas_call(
            kern,
            out_shape=jax.ShapeDtypeStruct((1, 1, M), A_x.dtype),
            in_specs=[pl.BlockSpec(memory_space=pl.ANY)] * 10,
            out_specs=pl.BlockSpec(memory_space=pltpu.VMEM),
            scratch_shapes=[
                pltpu.VMEM((1, 1, M), BF), pltpu.VMEM((4, 128), BF), pltpu.VMEM((64, 4, 32, DC), BF),
                head_buf, head_buf, head_buf, pltpu.VMEM((32, 4, 32, M), BF),
                ffn_buf, ffn_buf, ffn_buf, pltpu.VMEM((3, 4 * FT, M), BF),
                pltpu.VMEM((128, 128), F32), pltpu.VMEM((H, D), F32),
            ],
            compiler_params=pltpu.CompilerParams(vmem_limit_bytes=64 * 2**20, disable_bounds_checks=nochk),
        )(A_x, A_c_kv.reshape(4, SK // 4, DC), quarters(A_w_q), quarters(A_w_uk), quarters(A_w_uv),
          A_w_o.reshape(4, H * D // 4, M), B_w_r.reshape(4, 128), ffn_view(B_w_gate.T), ffn_view(B_w_up.T), ffn_view(B_w_down))

    return run


pallas_sequential_preLN__compressed_kv_cla__moe_arch_mod__decode_kernel = build()
```

```python
import jax
import jax.numpy as jnp
from jax import lax
from jax.experimental import pallas as pl
from jax.experimental.pallas import tpu as pltpu

H, D, M, DC, SK, F = 32, 128, 512, 512, 8192, 1376
BF, F32 = jnp.bfloat16, jnp.float32
NT = (((1,), (1,)), ((), ()))

NF = pl.cdiv(F, 128)
FT = F // 4 - 32 * (NF - 1)
F_ORDER = (10, 0, 5, 1, 6, 2, 7, 3, 8, 4, 9)

G_Q, G_UK, G_KV, G_UV, G_O, G_FFN = 0, 32, 64, 128, 160, 192
N_UNITS = G_FFN + 3 * NF
LEAD_LOW, LEAD_HIGH = 16, 6
ROWS = 8


def _aligned(i, n):
    return i if isinstance(i, int) else pl.multiple_of(i, n)


def _center(v):
    return v - jnp.mean(v, axis=-1, keepdims=True)


def _normalize(c):
    return c / jnp.sqrt(jnp.mean(c * c, axis=-1, keepdims=True) + 1e-5)


def _block(x_hbm, ckv_hbm, wq_hbm, wuk_hbm, wuv_hbm, wo_hbm, wr_hbm, wg_hbm, wu_hbm, wd_hbm, out_hbm,
           x_v, wr_v, ckv_v, wq_v, wuk_v, wuv_v, wo_v, wg_v, wu_v, wd_v, tail_v, r_v, ctx_v, out_v, sems):
    def quarters(src, rows, dst, cuts=(0, 3, 4)):
        return tuple((src.at[pl.ds(a, b - a), rows], dst.at[pl.ds(a, b - a)]) for a, b in zip(cuts, cuts[1:]))

    def head_unit(src, dst):
        return lambda c, d: quarters(src, pl.ds((c % 2) * 64 + (c // 2 + d) * 4, 4), dst.at[c + 2 * d])

    def ckv_unit(c, d):
        e = c // 2 + d
        r0 = _aligned((c % 2) * 512 + (e & 1) * 1024 + (e >> 1) * 32, 32)
        return quarters(ckv_hbm, pl.ds(r0, 32), ckv_v.at[c + 2 * d])

    def wo_unit(c, d):
        r0 = _aligned((c % 2) * 512 + (c // 2 + d) * 32, 32)
        return quarters(wo_hbm, pl.ds(r0, 32), wo_v.at[c + 2 * d])

    ffn = ((wg_hbm, wg_v), (wu_hbm, wu_v), (wd_hbm, wd_v))

    def ffn_unit(u, _):
        w, j = (u % 2, F_ORDER[u // 2]) if u < 2 * NF else (2, F_ORDER[u - 2 * NF])
        src, dst = ffn[w]
        if j == NF - 1:
            return tuple((src.at[k, pl.ds(j * 32, FT)], tail_v.at[w, pl.ds(k * FT, FT)]) for k in range(4))
        return quarters(src, pl.ds(j * 32, 32), dst.at[j], (0, 1, 2, 3, 4) if u == 3 * NF - 1 else (0, 3, 4))

    def ffn_tile(w, n):
        j = F_ORDER[n]
        return tail_v[w] if j == NF - 1 else ffn[w][1][j].reshape(128, M)

    segments = ((G_Q, head_unit(wq_hbm, wq_v)), (G_UK, head_unit(wuk_hbm, wuk_v)), (G_KV, ckv_unit),
                (G_UV, head_unit(wuv_hbm, wuv_v)), (G_O, wo_unit), (G_FFN, ffn_unit))

    def segment(g):
        return max(k for k, (base, _) in enumerate(segments) if base <= g)

    def copies(g, d=0):
        base, unit = segments[segment(g)]
        own_sem = g == N_UNITS - 1
        return [pltpu.make_async_copy(src, dst, sems.at[g + 2 * d + (n if own_sem else 0)])
                for n, (src, dst) in enumerate(unit(g - base, d))]

    def start_low(g, d=0):
        for c in copies(g, d)[:-1]:
            c.start(priority=1)

    def step(g, d=0):
        for c in copies(g, d):
            c.wait()
        if g + LEAD_HIGH < N_UNITS:
            copies(g + LEAD_HIGH, d)[-1].start(priority=0)
        if g + LEAD_LOW < N_UNITS:
            start_low(g + LEAD_LOW, d)

    def stage(g0, n_iter, per, fn, carry):
        def key(i):
            segs = tuple(segment(g0 + i * per + k + w) for k in range(per) for w in (0, LEAD_HIGH, LEAD_LOW))
            return i if len(segments) - 1 in segs else segs

        i = 0
        while i < n_iter:
            j = i + 1
            while j < n_iter and key(j) == key(i):
                j += 1
            g = g0 + i * per
            if j - i == 1:
                carry = fn(i, lambda k, g=g: step(g + k), carry)
            else:
                carry = lax.fori_loop(
                    i, j, lambda t, c, g=g, i=i: fn(t, lambda k: step(g + k, (t - i) * (per // 2)), c), carry)
            i = j
        return carry

    small = (pltpu.make_async_copy(x_hbm, x_v, sems.at[N_UNITS + 3]),
             pltpu.make_async_copy(wr_hbm, wr_v, sems.at[N_UNITS + 4]))
    start_low(0)
    for c in small:
        c.start()
    for g in range(LEAD_LOW):
        if g > 0:
            start_low(g)
        if g < LEAD_HIGH:
            copies(g)[-1].start(priority=int(g >= 3))

    row = lax.broadcasted_iota(jnp.int32, (H, 128), 0)
    lane = lax.broadcasted_iota(jnp.int32, (H, 128), 1)
    same_head = (lane % H) == row
    sublane = lax.broadcasted_iota(jnp.int32, (8, 128), 0)

    def head_tile(w_v, u, s):
        return w_v[u, :, s].reshape(4 * H, D)

    def tile_rows(i, p):
        return pl.ds(_aligned(p * 64 + i * 8, 8), 8)

    def spread(a):
        r_v[...] = jnp.concatenate([a[:, j * 128:(j + 1) * 128] for j in range(4)], axis=0).T

    def contract_latent(w_v):
        def fn(i, tick, acc):
            coef = [r_v[tile_rows(i, p), :] for p in range(2)]
            for k in range(4):
                tick(k)
                for s in range(4):
                    t = (k // 2) * 4 + s
                    lhs = jnp.where(same_head, coef[k % 2][t:t + 1, :], 0.0).astype(BF)
                    acc = acc + jnp.dot(lhs, head_tile(w_v, i * 4 + k, s), preferred_element_type=F32)
            return acc
        return fn

    for c in small:
        c.wait()
    x = x_v[0].astype(F32)
    spread(jnp.broadcast_to(_normalize(_center(x)), (H, M)))
    q = stage(G_Q, 8, 4, contract_latent(wq_v), jnp.zeros((H, D), F32)).astype(BF)

    def absorb(i, tick, carry):
        merged = [jnp.zeros((8, 128), F32)] * 2
        for k in range(4):
            tick(k)
            for s in range(4):
                o = lax.dot_general(q, head_tile(wuk_v, i * 4 + k, s), NT, preferred_element_type=F32)
                picked = jnp.sum(jnp.where(same_head, o, 0.0), axis=0, keepdims=True)
                merged[k % 2] = jnp.where(sublane == (k // 2) * 4 + s, picked, merged[k % 2])
        for p in range(2):
            r_v[tile_rows(i, p), :] = merged[p]
        return carry

    stage(G_UK, 8, 4, absorb, 0)
    step(G_KV)
    rt = r_v[...].T * (D ** -0.5)
    q_lat = jnp.concatenate([rt[j * H:(j + 1) * H, :] for j in range(4)], axis=1).astype(BF)

    def keys(u):
        return ckv_v[u].reshape(128, DC)

    def scores(u):
        return lax.dot_general(q_lat, keys(u), NT, preferred_element_type=F32)

    def softmax_update(s, m, l, acc):
        m_new = jnp.maximum(m, jnp.max(jnp.maximum(s[0], s[1]), axis=-1, keepdims=True))
        alpha = jnp.exp(m - m_new)
        p = [jnp.exp(v - m_new) for v in s]
        return [v.astype(BF) for v in p], m_new, alpha * l + p[0] + p[1], alpha * acc

    def add_values(i, p, acc):
        for k in range(2):
            acc = acc + jnp.dot(p[k], keys(2 * i + k), preferred_element_type=F32)
        return acc

    def attend(i, tick, carry):
        s, m, l, acc = carry
        tick(0)
        s_next = (scores(2 * i + 2), scores(2 * i + 3))
        p, m, l, acc = softmax_update(s, m, l, acc)
        tick(1)
        return s_next, m, l, add_values(i, p, acc)

    step(G_KV + 1)
    s0 = scores(0)
    step(G_KV + 2)
    carry = ((s0, scores(1)), jnp.full((H, 1), -jnp.inf, F32), jnp.zeros((H, 128), F32), jnp.zeros((H, DC), F32))
    carry = stage(G_KV + 3, 31, 2, attend, carry)
    step(G_UV + 1)
    p, _, l, acc = softmax_update(*carry)
    step(G_UV + 2)
    acc = add_values(31, p, acc)
    step(G_UV + 3)
    spread(acc / jnp.sum(l, axis=-1, keepdims=True))
    ctx = stage(G_UV + 4, 8, 4, contract_latent(wuv_v), jnp.zeros((H, D), F32))

    step(G_O + 4)
    for i in range(4):
        ctx_v[8 * i:8 * i + 8, :] = jnp.concatenate(
            [ctx[8 * j:8 * j + 8, 32 * i:32 * i + 32] for j in range(4)], axis=1)

    def project(g, tick, acc):
        for k in range(8):
            tick(k)
            lhs = jnp.broadcast_to(ctx_v[pl.ds(4 * k + g, 1), :], (ROWS, 128)).astype(BF)
            acc = acc + jnp.dot(lhs, wo_v[8 * g + k].reshape(128, M), preferred_element_type=F32)
        return acc

    attn = stage(G_O + 5, 4, 8, project, jnp.zeros((ROWS, M), F32))
    step(G_FFN + 5)
    h = x + attn[0:1, :]
    centered = _center(h)
    step(G_FFN + 6)
    hn = _normalize(centered)
    hb = jnp.broadcast_to(hn, (ROWS, M)).astype(BF)
    step(G_FFN + 7)
    wr = wr_v[...].astype(F32)
    wr = jnp.concatenate([wr[j:j + 1, :] for j in range(4)], axis=1)
    route = jax.nn.sigmoid(jnp.sum(hn * wr, axis=-1, keepdims=True))

    act, pre, g = [], None, G_FFN + 8
    for n in range(NF + 1):
        while g <= G_FFN + max(8 + n, min(2 * n + 1, 2 * NF)):
            step(g)
            g += 1
        if pre is not None:
            act.append(pre[0] * jax.nn.sigmoid(pre[0]) * pre[1])
        if n < NF:
            pre = [lax.dot_general(hb, ffn_tile(w, n), NT, preferred_element_type=F32) for w in range(2)]
    y = jnp.zeros((ROWS, M), F32)
    last = jnp.broadcast_to(act[-1][0:1, :] * route, (128, 128)).T
    for n in range(NF - 1):
        if n > 0:
            step(G_FFN + 2 * NF + n)
        y = y + jnp.dot(act[n].astype(BF), ffn_tile(2, n), preferred_element_type=F32)
    res = h + (hn + (hn * 0.0 + y[0:1, :] * route))

    part = jnp.where(lax.broadcasted_iota(jnp.int32, (8, M), 0) == 0, res, 0.0)
    pieces = copies(N_UNITS - 1)
    for k in (3, 0, 1, 2):
        pieces[k].wait()
        for r in range(0, 32, 8):
            a = jnp.concatenate([last[32 * k + r:32 * k + r + 8, :]] * (M // 128), axis=1)
            part = part + a * wd_v[F_ORDER[-1], k, r:r + 8, :].astype(F32)
    out_v[0] = jnp.sum(part, axis=0, keepdims=True).astype(out_v.dtype)
    store = pltpu.make_async_copy(out_v, out_hbm, sems.at[N_UNITS + 5])
    store.start()
    store.wait()


def _kernel(*refs):
    pl.run_scoped(lambda sems: _block(*refs, sems), pltpu.SemaphoreType.DMA((N_UNITS + 6,)))


@jax.jit
def pallas_sequential_preLN__compressed_kv_cla__moe_arch_mod__decode_kernel(
    A_x: jax.Array,
    A_c_kv: jax.Array,
    A_w_q: jax.Array,
    A_w_uk: jax.Array,
    A_w_uv: jax.Array,
    A_w_o: jax.Array,
    B_x: jax.Array,
    B_w_r: jax.Array,
    B_w_gate: jax.Array,
    B_w_up: jax.Array,
    B_w_down: jax.Array,
):
    del B_x
    head_view = lambda w: w.reshape(4, DC // 4, H, D)
    row_view = lambda w: w.reshape(4, -1, M)
    head_buf = pltpu.VMEM((32, 4, 4, H, D), BF)
    row_buf = lambda n: pltpu.VMEM((n, 4, 32, M), BF)
    return pl.pallas_call(
        _kernel,
        out_shape=jax.ShapeDtypeStruct((1, 1, M), A_x.dtype),
        in_specs=[pl.BlockSpec(memory_space=pl.ANY)] * 10,
        out_specs=pl.BlockSpec(memory_space=pl.ANY),
        scratch_shapes=[
            pltpu.VMEM((1, 1, M), BF), pltpu.VMEM((4, 128), BF), row_buf(64),
            head_buf, head_buf, head_buf, row_buf(32),
            row_buf(NF - 1), row_buf(NF - 1), row_buf(NF - 1), pltpu.VMEM((3, 4 * FT, M), BF),
            pltpu.VMEM((128, 128), F32), pltpu.VMEM((H, D), F32), pltpu.VMEM((1, 1, M), A_x.dtype),
        ],
        compiler_params=pltpu.CompilerParams(vmem_limit_bytes=64 * 2**20),
    )(A_x, row_view(A_c_kv), head_view(A_w_q), head_view(A_w_uk), head_view(A_w_uv), row_view(A_w_o),
      B_w_r.reshape(4, 128), row_view(B_w_gate.T), row_view(B_w_up.T), row_view(B_w_down))
```

```python
import jax
import jax.numpy as jnp
from jax import lax
from jax.experimental import pallas as pl
from jax.experimental.pallas import tpu as pltpu

H, D, M, DC, SK, F = 32, 128, 512, 512, 8192, 1376
BF, F32 = jnp.bfloat16, jnp.float32
NT = (((1,), (1,)), ((), ()))

NF = pl.cdiv(F, 128)
FT = F // 4 - 32 * (NF - 1)
F_ORDER = (10, 0, 5, 1, 6, 2, 7, 3, 8, 4, 9)

G_Q, G_UK, G_KV, G_UV, G_O, G_FFN = 0, 32, 64, 128, 160, 192
N_UNITS = G_FFN + 3 * NF
LEAD_LOW, LEAD_HIGH = 16, 6
ROWS = 8


def _aligned(i, n):
    return i if isinstance(i, int) else pl.multiple_of(i, n)


def _center(v):
    return v - jnp.mean(v, axis=-1, keepdims=True)


def _normalize(c):
    return c / jnp.sqrt(jnp.mean(c * c, axis=-1, keepdims=True) + 1e-5)


def _block(x_hbm, ckv_hbm, wq_hbm, wuk_hbm, wuv_hbm, wo_hbm, wr_hbm, wg_hbm, wu_hbm, wd_hbm, out_hbm,
           x_v, wr_v, ckv_v, wq_v, wuk_v, wuv_v, wo_v, wg_v, wu_v, wd_v, tail_v, r_v, ctx_v, out_v, sems):
    def quarters(src, rows, dst, cuts=(0, 3, 4)):
        return tuple((src.at[pl.ds(a, b - a), rows], dst.at[pl.ds(a, b - a)]) for a, b in zip(cuts, cuts[1:]))

    def head_unit(src, dst):
        return lambda c, d: quarters(src, pl.ds((c % 2) * 64 + (c // 2 + d) * 4, 4), dst.at[c + 2 * d])

    def ckv_unit(c, d):
        e = c // 2 + d
        r0 = _aligned((c % 2) * 512 + (e & 1) * 1024 + (e >> 1) * 32, 32)
        return quarters(ckv_hbm, pl.ds(r0, 32), ckv_v.at[c + 2 * d])

    def wo_unit(c, d):
        r0 = _aligned((c % 2) * 512 + (c // 2 + d) * 32, 32)
        return quarters(wo_hbm, pl.ds(r0, 32), wo_v.at[c + 2 * d])

    ffn = ((wg_hbm, wg_v), (wu_hbm, wu_v), (wd_hbm, wd_v))

    def ffn_unit(u, _):
        w, j = (u % 2, F_ORDER[u // 2]) if u < 2 * NF else (2, F_ORDER[u - 2 * NF])
        src, dst = ffn[w]
        if j == NF - 1:
            return tuple((src.at[k, pl.ds(j * 32, FT)], tail_v.at[w, pl.ds(k * FT, FT)]) for k in range(4))
        return quarters(src, pl.ds(j * 32, 32), dst.at[j], (0, 1, 2, 3, 4) if u == 3 * NF - 1 else (0, 3, 4))

    def ffn_tile(w, n):
        j = F_ORDER[n]
        return tail_v[w] if j == NF - 1 else ffn[w][1][j].reshape(128, M)

    segments = ((G_Q, head_unit(wq_hbm, wq_v)), (G_UK, head_unit(wuk_hbm, wuk_v)), (G_KV, ckv_unit),
                (G_UV, head_unit(wuv_hbm, wuv_v)), (G_O, wo_unit), (G_FFN, ffn_unit))

    def segment(g):
        return max(k for k, (base, _) in enumerate(segments) if base <= g)

    def copies(g, d=0):
        base, unit = segments[segment(g)]
        own_sem = g == N_UNITS - 1
        return [pltpu.make_async_copy(src, dst, sems.at[g + 2 * d + (n if own_sem else 0)])
                for n, (src, dst) in enumerate(unit(g - base, d))]

    def start_low(g, d=0):
        for c in copies(g, d)[:-1]:
            c.start(priority=1)

    def arrive(g, d=0):
        for c in copies(g, d):
            c.wait()

    def refill(g, d=0):
        if g + LEAD_HIGH < N_UNITS:
            copies(g + LEAD_HIGH, d)[-1].start(priority=0)
        if g + LEAD_LOW < N_UNITS:
            start_low(g + LEAD_LOW, d)

    def step(g, d=0):
        arrive(g, d)
        refill(g, d)

    def stage(g0, n_iter, per, fn, carry):
        def key(i):
            segs = tuple(segment(g0 + i * per + k + w) for k in range(per) for w in (0, LEAD_HIGH, LEAD_LOW))
            return i if len(segments) - 1 in segs else segs

        i = 0
        while i < n_iter:
            j = i + 1
            while j < n_iter and key(j) == key(i):
                j += 1
            g = g0 + i * per
            if j - i == 1:
                carry = fn(i, lambda k, g=g: (g + k, 0), carry)
            else:
                carry = lax.fori_loop(
                    i, j, lambda t, c, g=g, i=i: fn(t, lambda k: (g + k, (t - i) * (per // 2)), c), carry)
            i = j
        return carry

    small = (pltpu.make_async_copy(x_hbm, x_v, sems.at[N_UNITS + 3]),
             pltpu.make_async_copy(wr_hbm, wr_v, sems.at[N_UNITS + 4]))
    start_low(0)
    for c in small:
        c.start()
    for g in range(LEAD_LOW):
        if g > 0:
            start_low(g)
        if g < LEAD_HIGH:
            copies(g)[-1].start(priority=int(g >= 3))

    row = lax.broadcasted_iota(jnp.int32, (H, 128), 0)
    lane = lax.broadcasted_iota(jnp.int32, (H, 128), 1)
    same_head = (lane % H) == row
    sublane = lax.broadcasted_iota(jnp.int32, (8, 128), 0)

    def head_tile(w_v, u, s):
        return w_v[u, :, s].reshape(4 * H, D)

    def tile_rows(i, p):
        return pl.ds(_aligned(p * 64 + i * 8, 8), 8)

    def spread(a):
        r_v[...] = jnp.concatenate([a[:, j * 128:(j + 1) * 128] for j in range(4)], axis=0).T

    def contract_latent(w_v):
        def fn(i, at, acc):
            coef = [r_v[tile_rows(i, p), :] for p in range(2)]
            for k in range(4):
                step(*at(k))
                for s in range(4):
                    t = (k // 2) * 4 + s
                    lhs = jnp.where(same_head, coef[k % 2][t:t + 1, :], 0.0).astype(BF)
                    acc = acc + jnp.dot(lhs, head_tile(w_v, i * 4 + k, s), preferred_element_type=F32)
            return acc
        return fn

    for c in small:
        c.wait()
    x = x_v[0].astype(F32)
    spread(jnp.broadcast_to(_normalize(_center(x)), (H, M)))
    q = stage(G_Q, 8, 4, contract_latent(wq_v), jnp.zeros((H, D), F32)).astype(BF)

    def absorb(i, at, carry):
        merged = [jnp.zeros((8, 128), F32)] * 2
        for k in range(4):
            step(*at(k))
            for s in range(4):
                o = lax.dot_general(q, head_tile(wuk_v, i * 4 + k, s), NT, preferred_element_type=F32)
                picked = jnp.sum(jnp.where(same_head, o, 0.0), axis=0, keepdims=True)
                merged[k % 2] = jnp.where(sublane == (k // 2) * 4 + s, picked, merged[k % 2])
        for p in range(2):
            r_v[tile_rows(i, p), :] = merged[p]
        return carry

    stage(G_UK, 8, 4, absorb, 0)
    step(G_KV)
    rt = r_v[...].T * (D ** -0.5)
    q_lat = jnp.concatenate([rt[j * H:(j + 1) * H, :] for j in range(4)], axis=1).astype(BF)

    def keys(u):
        return ckv_v[u].reshape(128, DC)

    def scores(u):
        return lax.dot_general(q_lat, keys(u), NT, preferred_element_type=F32)

    def softmax_update(s, m, l, acc):
        m_new = jnp.maximum(m, jnp.max(jnp.maximum(s[0], s[1]), axis=-1, keepdims=True))
        alpha = jnp.exp(m - m_new)
        p = [jnp.exp(v - m_new) for v in s]
        return [v.astype(BF) for v in p], m_new, alpha * l + p[0] + p[1], alpha * acc

    def values(p, u):
        return jnp.dot(p, keys(u), preferred_element_type=F32)

    def attend(i, at, carry):
        s, m, l, acc = carry
        arrive(*at(0))
        arrive(*at(1))
        refill(*at(0))
        s_next = (scores(2 * i + 2), scores(2 * i + 3))
        p, m, l, acc = softmax_update(s, m, l, acc)
        acc = acc + values(p[0], 2 * i)
        refill(*at(1))
        return s_next, m, l, acc + values(p[1], 2 * i + 1)

    step(G_KV + 1)
    s0 = scores(0)
    step(G_KV + 2)
    carry = ((s0, scores(1)), jnp.full((H, 1), -jnp.inf, F32), jnp.zeros((H, 128), F32), jnp.zeros((H, DC), F32))
    carry = stage(G_KV + 3, 31, 2, attend, carry)
    step(G_UV + 1)
    p, _, l, acc = softmax_update(*carry)
    step(G_UV + 2)
    acc = acc + values(p[0], 62) + values(p[1], 63)
    step(G_UV + 3)
    spread(acc / jnp.sum(l, axis=-1, keepdims=True))
    ctx = stage(G_UV + 4, 8, 4, contract_latent(wuv_v), jnp.zeros((H, D), F32))

    step(G_O + 4)
    for i in range(4):
        ctx_v[8 * i:8 * i + 8, :] = jnp.concatenate(
            [ctx[8 * j:8 * j + 8, 32 * i:32 * i + 32] for j in range(4)], axis=1)

    def project(g, at, acc):
        for k in range(8):
            step(*at(k))
            lhs = jnp.broadcast_to(ctx_v[pl.ds(4 * k + g, 1), :], (ROWS, 128)).astype(BF)
            acc = acc + jnp.dot(lhs, wo_v[8 * g + k].reshape(128, M), preferred_element_type=F32)
        return acc

    attn = stage(G_O + 5, 4, 8, project, jnp.zeros((ROWS, M), F32))
    step(G_FFN + 5)
    h = x + attn[0:1, :]
    centered = _center(h)
    step(G_FFN + 6)
    hn = _normalize(centered)
    hb = jnp.broadcast_to(hn, (ROWS, M)).astype(BF)
    step(G_FFN + 7)
    wr = wr_v[...].astype(F32)
    wr = jnp.concatenate([wr[j:j + 1, :] for j in range(4)], axis=1)
    route = jax.nn.sigmoid(jnp.sum(hn * wr, axis=-1, keepdims=True))

    act, pre, g = [], None, G_FFN + 8
    for n in range(NF + 1):
        while g <= G_FFN + max(8 + n, min(2 * n + 1, 2 * NF)):
            step(g)
            g += 1
        if pre is not None:
            act.append(pre[0] * jax.nn.sigmoid(pre[0]) * pre[1])
        if n < NF:
            pre = [lax.dot_general(hb, ffn_tile(w, n), NT, preferred_element_type=F32) for w in range(2)]
    y = jnp.zeros((ROWS, M), F32)
    last = jnp.broadcast_to(act[-1][0:1, :] * route, (128, 128)).T
    for n in range(NF - 1):
        if n > 0:
            step(G_FFN + 2 * NF + n)
        y = y + jnp.dot(act[n].astype(BF), ffn_tile(2, n), preferred_element_type=F32)
    res = h + (hn + (hn * 0.0 + y[0:1, :] * route))

    part = jnp.where(lax.broadcasted_iota(jnp.int32, (8, M), 0) == 0, res, 0.0)
    pieces = copies(N_UNITS - 1)
    for k in (3, 0, 1, 2):
        pieces[k].wait()
        for r in range(0, 32, 8):
            a = jnp.concatenate([last[32 * k + r:32 * k + r + 8, :]] * (M // 128), axis=1)
            part = part + a * wd_v[F_ORDER[-1], k, r:r + 8, :].astype(F32)
    out_v[0] = jnp.sum(part, axis=0, keepdims=True).astype(out_v.dtype)
    store = pltpu.make_async_copy(out_v, out_hbm, sems.at[N_UNITS + 5])
    store.start()
    store.wait()


def _kernel(*refs):
    pl.run_scoped(lambda sems: _block(*refs, sems), pltpu.SemaphoreType.DMA((N_UNITS + 6,)))


@jax.jit
def pallas_sequential_preLN__compressed_kv_cla__moe_arch_mod__decode_kernel(
    A_x: jax.Array,
    A_c_kv: jax.Array,
    A_w_q: jax.Array,
    A_w_uk: jax.Array,
    A_w_uv: jax.Array,
    A_w_o: jax.Array,
    B_x: jax.Array,
    B_w_r: jax.Array,
    B_w_gate: jax.Array,
    B_w_up: jax.Array,
    B_w_down: jax.Array,
):
    del B_x
    head_view = lambda w: w.reshape(4, DC // 4, H, D)
    row_view = lambda w: w.reshape(4, -1, M)
    head_buf = pltpu.VMEM((32, 4, 4, H, D), BF)
    row_buf = lambda n: pltpu.VMEM((n, 4, 32, M), BF)
    return pl.pallas_call(
        _kernel,
        out_shape=jax.ShapeDtypeStruct((1, 1, M), A_x.dtype),
        in_specs=[pl.BlockSpec(memory_space=pl.ANY)] * 10,
        out_specs=pl.BlockSpec(memory_space=pl.ANY),
        scratch_shapes=[
            pltpu.VMEM((1, 1, M), BF), pltpu.VMEM((4, 128), BF), row_buf(64),
            head_buf, head_buf, head_buf, row_buf(32),
            row_buf(NF - 1), row_buf(NF - 1), row_buf(NF - 1), pltpu.VMEM((3, 4 * FT, M), BF),
            pltpu.VMEM((128, 128), F32), pltpu.VMEM((H, D), F32), pltpu.VMEM((1, 1, M), A_x.dtype),
        ],
        compiler_params=pltpu.CompilerParams(vmem_limit_bytes=64 * 2**20),
    )(A_x, row_view(A_c_kv), head_view(A_w_q), head_view(A_w_uk), head_view(A_w_uv), row_view(A_w_o),
      B_w_r.reshape(4, 128), row_view(B_w_gate.T), row_view(B_w_up.T), row_view(B_w_down))
```
